```python
import os as _os
_os.environ.setdefault("JAX_PLATFORMS", "cpu")
import jax
import jax.numpy as jnp

def _softmax(x, axis=-1):
    return jax.nn.softmax(x, axis=axis)
def _gelu(x):
    return jax.nn.gelu(x, approximate=True)
def _silu(x):
    return jax.nn.silu(x)
def _sigmoid(x):
    return jax.nn.sigmoid(x)
def _layernorm(x, axis=-1, eps=1e-5):
    m = jnp.mean(x, axis=axis, keepdims=True)
    v = jnp.var(x, axis=axis, keepdims=True)
    return (x - m) / jnp.sqrt(v + eps)
def _scatter_add(tgt, idx, src, axis=0):
    return tgt.at[idx].add(src)
def _segment_sum(src, seg, n):
    return jax.ops.segment_sum(src, seg, n)
class _Rng:
    def __init__(self, key):
        self._k = key
    def _next(self):
        self._k, sub = jax.random.split(self._k)
        return sub
    def normal(self, shape):
        return jax.random.normal(self._next(), shape, dtype=jnp.bfloat16)
    def randint(self, lo, hi, shape):
        return jax.random.randint(self._next(), shape, lo, hi, dtype=jnp.int32)
    def uniform(self, shape, lo=0.0, hi=1.0):
        return jax.random.uniform(self._next(), shape, jnp.bfloat16, lo, hi)
    def permutation(self, n):
        return jax.random.permutation(self._next(), n)


kernel_name = 'sequential_preLN__sliding_block__swiglu_ffn__prompt'

def setup_inputs():
    _rng = _Rng(jax.random.key(int.from_bytes(__import__("os").urandom(4), "little")))
    _w = (lambda a: (lambda t: t.astype(jnp.bfloat16) if jnp.issubdtype(t.dtype, jnp.floating) else t)(jnp.asarray(a)))
    def _A_setup():
        B, S, D = 1, 2048, 512
        return {
            "x": _w((lambda *s: _rng.normal(s) * 0.05)(B, S, D)),
            "wqkv": _w((lambda *s: _rng.normal(s) * 0.05)(D, 3 * D)),
            "wo": _w((lambda *s: _rng.normal(s) * 0.05)(D, D)),
        }
    _A_in = _A_setup()

    def _B_setup():
        B, S, D, F = 1, 2048, 512, 1792
        return {
            "x": _w((lambda *s: _rng.normal(s) * 0.05)(B, S, D)),
            "w_gate": _w((lambda *s: _rng.normal(s) * 0.05)(D, F)),
            "w_up": _w((lambda *s: _rng.normal(s) * 0.05)(D, F)),
            "w_down": _w((lambda *s: _rng.normal(s) * 0.05)(F, D)),
        }
    _B_in = _B_setup()

    return {
        "A_x": _A_in["x"],
        "A_wqkv": _A_in["wqkv"],
        "A_wo": _A_in["wo"],
        "B_x": _B_in["x"],
        "B_w_gate": _B_in["w_gate"],
        "B_w_up": _B_in["w_up"],
        "B_w_down": _B_in["w_down"],
    }

def reference(A_x, A_wqkv, A_wo, B_x, B_w_gate, B_w_up, B_w_down):
    def _A_ref(x, wqkv, wo):
        B, S, D = x.shape
        H = 32; Dh = D // H; W = 256
        qkv = (lambda x, *d: x.transpose(*d))((x @ wqkv).reshape(B, S, 3, H, Dh), 2, 0, 3, 1, 4)
        q, k, v = qkv[0], qkv[1], qkv[2]
        scores = jnp.einsum("bhqd,bhkd->bhqk", q, k) * (Dh ** -0.5)
        idx = jnp.arange(S)
        mask = (idx[:, None] - idx[None, :] >= 0) & (idx[:, None] - idx[None, :] < W)
        scores = jnp.where(mask[None, None], scores, -1e9)
        p = _softmax(scores, axis=-1)
        o = jnp.einsum("bhqk,bhkd->bhqd", p, v)
        return (lambda x, *d: x.transpose(*d))(o, 0, 2, 1, 3).reshape(B, S, D) @ wo

    def _B_ref(x, w_gate, w_up, w_down):
        g = _silu(x @ w_gate)
        u = x @ w_up
        return (g * u) @ w_down

    x = A_x
    h = x + _A_ref(_layernorm(x, axis=-1), A_wqkv, A_wo)
    h2 = h + _B_ref(_layernorm(h, axis=-1), B_w_gate, B_w_up, B_w_down)
    return h2
```

```python
import functools
import numpy as np
import jax
import jax.numpy as jnp
from jax import lax
import jax.experimental.pallas as pl
import jax.experimental.pallas.tpu as pltpu

S, D, F, H, DH, W = 2048, 512, 1792, 32, 16, 256
TM = 256
NB = S // TM
QB = 64
EPS = 1e-5
QSCALE = float(DH ** -0.5 * np.log2(np.e))
F32, BF16, U32 = jnp.float32, jnp.bfloat16, jnp.uint32
NT = (((1,), (1,)), ((), ()))
CFG = dict(order="mix", fc=256)


def _ln(x):
    m = jnp.mean(x, axis=-1, keepdims=True)
    c = x - m
    v = jnp.mean(c * c, axis=-1, keepdims=True)
    return c * lax.rsqrt(v + EPS)


def _band(x, m):
    return pltpu.bitcast(pltpu.bitcast(x, U32) & m, BF16)


def _kernel(x_hbm, wqkv_hbm, wo_hbm, wg_hbm, wu_hbm, wd_hbm, out_hbm,
            x_s, wqkv_s, wo_s, wg_s, wu_s, wd_s, out_s, q_s, k_s, vt_s, ot_s, h_s, hn_s, a_s, sems, osems):
    def xcopy(lo, n, sem):
        return pltpu.make_async_copy(x_hbm.at[pl.ds(lo, n)], x_s.at[pl.ds(lo, n)], sems.at[sem])
    c_x0 = xcopy(0, TM, 0)
    c_x1 = xcopy(TM, S - TM, 1)
    c_w = [pltpu.make_async_copy(a, b, sems.at[2 + n]) for n, (a, b) in enumerate(
        [(wqkv_hbm, wqkv_s), (wo_hbm, wo_s), (wg_hbm, wg_s), (wu_hbm, wu_s), (wd_hbm, wd_s)])]
    c_x0.start(); c_w[0].start(); c_x1.start()
    for c in c_w[1:]:
        c.start()

    def ocopy(b):
        r = pl.ds(pl.multiple_of(b * TM, TM), TM)
        return pltpu.make_async_copy(out_s.at[r], out_hbm.at[r], osems.at[b])

    lane = lax.broadcasted_iota(jnp.int32, (1, 128), 1)
    head_mask = [jnp.where(lane // DH == h, np.uint32(0xFFFFFFFF), np.uint32(0)) for h in range(8)]
    lo_half = lane < QB
    row = lax.broadcasted_iota(jnp.int32, (QB, 128), 0)
    col = lax.broadcasted_iota(jnp.int32, (QB, 128), 1) % QB
    new_tri = row <= col
    new_bits = pltpu.bitcast(jnp.where(new_tri, 1.0, 0.0).astype(BF16), U32)
    new_bits = (new_bits >> 7) & np.uint32(0x00010001)
    new_bits = (new_bits << 16) - new_bits
    old_bits = ~new_bits

    def attn_tasks(b, first):
        r0 = 0 if first else pl.multiple_of(b * TM, TM)
        st = {}

        def t_ln():
            st["xn"] = _ln(x_s[pl.ds(r0, TM), :].astype(F32)).astype(BF16)

        def t_q():
            q = jnp.dot(st["xn"], wqkv_s[:, 0:D], preferred_element_type=F32)
            q_s[...] = (q * QSCALE).astype(BF16)

        def t_k():
            k = jnp.dot(st["xn"], wqkv_s[:, D:2 * D], preferred_element_type=F32)
            k_s[pl.ds(r0, TM), :] = k.astype(BF16)

        def t_v():
            v = jnp.dot(st["xn"], wqkv_s[:, 2 * D:3 * D], preferred_element_type=F32)
            for m in range(TM // 128):
                vt_s[b * (TM // 128) + m] = v[128 * m:128 * (m + 1), :].T.astype(BF16)

        pre = [t_ln, t_k, t_v, t_q]

        def t_qk(j, g):
            def run():
                qt = q_s[QB * j:QB * (j + 1), 128 * g:128 * (g + 1)]
                hs = [2 * p + (e ^ (j & 1)) for p in range(4) for e in range(2)]
                qbd = jnp.concatenate([_band(qt, head_mask[h]) for h in hs], axis=0)
                if first:
                    kk = k_s[0:QB * (j + 1), 128 * g:128 * (g + 1)]
                else:
                    kk = k_s[pl.ds(pl.multiple_of(r0 + QB * j - W, QB), W + QB), 128 * g:128 * (g + 1)]
                st["s", j, g] = lax.dot_general(kk, qbd, NT, preferred_element_type=F32)
            return run

        def t_sm(j, g, p):
            def run():
                s = st["s", j, g][:, 128 * p:128 * (p + 1)]
                n = s.shape[0]
                if first:
                    edge = jnp.where(new_tri, s[n - QB:], -1e9)
                    parts = [edge] + ([s[:n - QB]] if n > QB else [])
                else:
                    edge = jnp.where(new_tri, s[W:], s[:QB])
                    parts = [edge, s[QB:W]]
                s = jnp.concatenate(parts, axis=0)
                e = jnp.exp2(s - jnp.max(s, axis=0, keepdims=True))
                st["l", j, g, p] = jnp.sum(e, axis=0, keepdims=True)
                e = e.astype(BF16)
                ee = e[:QB]
                blocks = ([] if first else [_band(ee, old_bits)]) + ([e[QB:]] if e.shape[0] > QB else [])
                blocks.append(ee if first else _band(ee, new_bits))
                z = jnp.zeros((QB, 128), BF16)
                if j & 1:
                    blocks = blocks if first else [z] + blocks
                else:
                    blocks = blocks + [z]
                st["p", j, g, p] = jnp.concatenate(blocks, axis=0)
            return run

        def t_pv(j, g, p):
            def run():
                pt = st.pop(("p", j, g, p))
                nt = pt.shape[0] // 128
                m1 = b * (TM // 128) + j // 2
                rows = slice(128 * g + 32 * p, 128 * g + 32 * (p + 1))
                vt = jnp.concatenate([vt_s[m1 - (nt - 1) + t, rows, :] for t in range(nt)], axis=1)
                o = jnp.dot(vt, pt, preferred_element_type=F32)
                lo, hi = (o[DH:], o[:DH]) if j & 1 else (o[:DH], o[DH:])
                z = jnp.where(lo_half, lo, hi) * pl.reciprocal(st.pop(("l", j, g, p)), approx=False)
                if j & 1:
                    ze = st.pop(("z", g, p))
                    c = slice(128 * (j // 2), 128 * (j // 2 + 1))
                    ot_s[128 * g + 32 * p:128 * g + 32 * p + DH, c] = jnp.where(lo_half, ze, z)
                    ot_s[128 * g + 32 * p + DH:128 * g + 32 * (p + 1), c] = pltpu.roll(jnp.where(lo_half, z, ze), QB, 1)
                else:
                    st["z", g, p] = z
            return run

        units = [(j, g) for jj in range(TM // 128) for g in range(4) for j in (2 * jj, 2 * jj + 1)]
        steps = []
        for n in range(len(units) + 1):
            ts = []
            if n < len(units):
                ts.append(t_qk(*units[n]))
            if n >= 1:
                for p in range(4):
                    ts += [t_sm(*units[n - 1], p), t_pv(*units[n - 1], p)]
            steps.append(ts)

        def t_o():
            o = ot_s[...].T.astype(BF16)
            h = x_s[pl.ds(r0, TM), :].astype(F32) + jnp.dot(o, wo_s[...], preferred_element_type=F32)
            h_s[...] = h
            hn_s[...] = _ln(h).astype(BF16)
        return pre, steps, t_o

    def ffn_tasks(b):
        r0 = pl.multiple_of(b * TM, TM)
        fc = CFG["fc"]
        ts = []

        def t_gu(c):
            def run():
                cs = slice(fc * c, fc * (c + 1))
                hn = hn_s[...]
                g = jnp.dot(hn, wg_s[:, cs], preferred_element_type=F32)
                u = jnp.dot(hn, wu_s[:, cs], preferred_element_type=F32)
                hg = 0.5 * g
                a_s[:, cs] = ((hg + hg * jnp.tanh(hg)) * u).astype(BF16)
            return run

        def t_d(c):
            def run():
                cs = slice(128 * c, 128 * (c + 1))
                y = jnp.dot(a_s[...], wd_s[:, cs], preferred_element_type=F32)
                out_s[pl.ds(r0, TM), cs] = (h_s[:, cs] + y).astype(out_s.dtype)
            return run
        return [t_gu(c) for c in range(F // fc)] + [t_d(c) for c in range(D // 128)]

    c_x0.wait(); c_w[0].wait()
    pre, steps, t_o = attn_tasks(0, True)
    for t in pre + [t for ts in steps for t in ts]:
        t()
    c_w[1].wait()
    t_o()
    c_x1.wait()
    for c in c_w[2:]:
        c.wait()

    def body(b, carry):
        pre, steps, t_o = attn_tasks(b, False)
        ft = ffn_tasks(b - 1)
        if CFG["order"] == "seq":
            for t in ft + pre + [t for ts in steps for t in ts]:
                t()
        else:
            for t in pre:
                t()
            done = 0
            for n, ts in enumerate(steps):
                for t in ts:
                    t()
                want = (n + 1) * len(ft) // len(steps)
                while done < want:
                    ft[done](); done += 1
        t_o()
        ocopy(b - 1).start()
        return carry
    lax.fori_loop(1, NB, body, 0)
    for t in ffn_tasks(NB - 1):
        t()
    ocopy(NB - 1).start()
    for b in range(NB):
        ocopy(b).wait()


@jax.jit
def pallas_sequential_preLN__sliding_block__swiglu_ffn__prompt_kernel(A_x, A_wqkv, A_wo, B_x, B_w_gate, B_w_up, B_w_down):
    del B_x
    any_spec = pl.BlockSpec(memory_space=pl.ANY)
    out = pl.pallas_call(
        _kernel,
        out_shape=jax.ShapeDtypeStruct((S, D), A_x.dtype),
        in_specs=[any_spec] * 6,
        out_specs=any_spec,
        scratch_shapes=[
            pltpu.VMEM((S, D), BF16), pltpu.VMEM((D, 3 * D), BF16), pltpu.VMEM((D, D), BF16),
            pltpu.VMEM((D, F), BF16), pltpu.VMEM((D, F), BF16), pltpu.VMEM((F, D), BF16),
            pltpu.VMEM((S, D), A_x.dtype),
            pltpu.VMEM((TM, D), BF16), pltpu.VMEM((S, D), BF16), pltpu.VMEM((S // 128, D, 128), BF16),
            pltpu.VMEM((D, TM), F32), pltpu.VMEM((TM, D), F32), pltpu.VMEM((TM, D), BF16), pltpu.VMEM((TM, F), BF16),
            pltpu.SemaphoreType.DMA((7,)), pltpu.SemaphoreType.DMA((NB,)),
        ],
        compiler_params=pltpu.CompilerParams(vmem_limit_bytes=64 * 1024 * 1024),
    )(A_x.reshape(S, D), A_wqkv, A_wo, B_w_gate, B_w_up, B_w_down)
    return out.reshape(1, S, D)
```

```python
import contextlib
import numpy as np
import jax
import jax.numpy as jnp
from jax import lax
import jax.experimental.pallas as pl
import jax.experimental.pallas.tpu as pltpu

S, D, F, H, DH, W = 2048, 512, 1792, 32, 16, 256
EPS = 1e-5
QSCALE = float(DH ** -0.5 * np.log2(np.e))
F32, BF16, U32 = jnp.float32, jnp.bfloat16, jnp.uint32
CFG = dict(tm=256, lag=0, ahead=8, qs=4, smpos=1, st='qogd', grp=2, sord=1, maxpos=1, sumpos=0, pm=1, pg=1, pd=0, pq=1, po=0, pre=3, mid=4, rval=1, pcost=0, pa=1, q0=1, o0=0, g0=0, d0=0, tail=3, flags={'XLA_TPU_FORCE_LP_LLO_SCHEDULER': True})


def _scope(n):
    return jax.named_scope("z_" + n) if CFG.get("scopes") else contextlib.nullcontext()


def _ln(x):
    m = jnp.mean(x, axis=-1, keepdims=True)
    c = x - m
    v = jnp.mean(c * c, axis=-1, keepdims=True)
    return c * lax.rsqrt(v + EPS)


def _u32(x):
    return pltpu.bitcast(x.astype(BF16), U32)


def _bf(x):
    return pltpu.bitcast(x, BF16)


def _dot(a, b):
    return jnp.dot(a, b, preferred_element_type=F32)


def _strassen_lhs(a11, a12, a21, a22):
    return [a11 + a22, a21 + a22, a11, a22, a11 + a12, a21 - a11, a12 - a22]


def _strassen_rhs(b11, b12, b21, b22, scale1=None):
    f11, f12, f21, f22 = [b.astype(F32) for b in (b11, b12, b21, b22)]
    if scale1 is not None:
        b11 = f11 = f11 * scale1
        f21 = f21 * scale1
    return [f11 + f22, b11, f12 - f22, f21 - f11, b22, f11 + f12, f21 + f22]


def _strassen_steps(prod, emit):
    if CFG["sord"]:
        c = {}

        def s61():
            m6 = prod(5)
            c[1] = prod(0)
            c["t"] = c[1] + m6

        def s23():
            c[2], c[3] = prod(1), prod(2)
            c[22] = c.pop("t") - c[2] + c[3]

        def s47():
            m4 = prod(3)
            c["u"] = c.pop(1) + m4 + prod(6)
            emit(1, c.pop(2) + m4, c.pop(22))

        def s5():
            m5 = prod(4)
            emit(0, c.pop("u") - m5, c.pop(3) + m5)
        return [(s61, 2), (s23, 2), (s47, 2), (s5, 1)]
    c = {}

    def s6():
        c[22] = prod(5)

    def s7():
        c[11] = prod(6)

    def s1():
        m = prod(0)
        c[11] += m
        c[22] += m

    def s2():
        c[21] = prod(1)
        c[22] -= c[21]

    def s3():
        c[12] = prod(2)
        c[22] += c[12]

    def s4():
        m = prod(3)
        c[11] += m
        emit(1, c.pop(21) + m, c.pop(22))

    def s5():
        m = prod(4)
        emit(0, c.pop(11) - m, c.pop(12) + m)
    return [(f, 1) for f in (s6, s7, s1, s2, s3, s4, s5)]


def _kernel(x_hbm, wqkv_hbm, wo_hbm, wg_hbm, wu_hbm, wd_hbm, out_hbm,
            x_s, wqkv_s, wo_s, wg_s, wu_s, wd_s, out_s,
            qt_s, k_s, ks_s, vt_s, ot_s, h_s, rq_s, ro_s, rg_s, rd_s, sems, osems):
    TM = CFG['tm']
    NB, HM, NT_ = S // TM, TM // 2, TM // 128
    nsem = [0]

    def copy(src, dst):
        nsem[0] += 1
        return pltpu.make_async_copy(src, dst, sems.at[nsem[0] - 1])

    def rows(b, n=1):
        return pl.ds(b * TM, n * TM)

    def cols(src, dst, lo, n):
        return copy(src.at[:, pl.ds(lo, n)], dst.at[:, pl.ds(lo, n)])
    c_x0, c_x1, c_x2 = [copy(x_hbm.at[r], x_s.at[r]) for r in (rows(0), rows(1, 1 + CFG['pa']), rows(2 + CFG['pa'], NB - 2 - CFG['pa']))]
    c_qkv = [[cols(wqkv_hbm, wqkv_s, D * w + 256 * c, 256) for w in range(3)] for c in range(2)]
    c_wo, c_wd = copy(wo_hbm, wo_s), copy(wd_hbm, wd_s)
    c_wg, c_wu = copy(wg_hbm, wg_s), copy(wu_hbm, wu_s)

    def ocopy(b, c):
        if b < NB - 1:
            return pltpu.make_async_copy(out_s.at[rows(b)], out_hbm.at[rows(b)], osems.at[b])
        cs = pl.ds(256 * c, 256)
        return pltpu.make_async_copy(out_s.at[rows(b), cs], out_hbm.at[rows(b), cs], osems.at[b + c])

    ONES, ZERO = np.uint32(0xFFFFFFFF), np.uint32(0)
    lane = lax.broadcasted_iota(jnp.int32, (1, 128), 1)
    quad = lane // 32
    quad_bits = [jnp.where(quad == g, ONES, ZERO) for g in range(4)]
    late = lane >= 64
    row = lax.broadcasted_iota(jnp.int32, (64, 128), 0)
    col = lax.broadcasted_iota(jnp.int32, (64, 128), 1) % 64
    new_tri = row <= col
    st, pending = {}, []

    def ch(c):
        return slice(128 * c, 128 * (c + 1))

    def group(steps, cost):
        n = CFG["grp"]
        return [((lambda ss=steps[k:k + n]: [f() for f, _ in ss] and None), cost * sum(w for _, w in steps[k:k + n]))
                for k in range(0, len(steps), n)]

    def put_lhs(name, a):
        st[name] = [l.astype(BF16) for l in _strassen_lhs(
            a[:HM, :D // 2], a[:HM, D // 2:], a[HM:, :D // 2], a[HM:, D // 2:])]

    def prep_rhs(ref, k, c, *quads):
        def run():
            for i, r in enumerate(_strassen_rhs(*[q() for q in quads], scale1=None)):
                if CFG["rval"]:
                    st["r", id(ref), i, k.start, c] = r.astype(BF16)
                else:
                    ref[i, k, ch(c)] = _u32(r)
        return (run, CFG["pcost"])

    def rhs(ref, i, c, k=slice(None)):
        return st["r", id(ref), i, k.start, c] if CFG["rval"] else _bf(ref[i, k, ch(c)])

    def prep_cols(ref, c, w1, c1, w2, c2):
        lo, hi = slice(0, D // 2), slice(D // 2, D)
        return prep_rhs(ref, slice(None), c, lambda: w1[lo, ch(c1)], lambda: w2[lo, ch(c2)],
                        lambda: w1[hi, ch(c1)], lambda: w2[hi, ch(c2)])

    def proj_tasks(b):
        fast = "q" in CFG["st"] and b >= CFG["q0"]

        def t_ln():
            xn = _ln(x_s[rows(b), :].astype(F32))
            if fast:
                put_lhs("lx", xn)
            else:
                st["xn"] = xn.astype(BF16)

        def emit(which, c, r, y):
            m0 = NT_ * b + NT_ // 2 * r
            if which == 1:
                k_s[64 * m0:64 * m0 + HM // 2, ch(c)] = _u32(y)
            for m in range(m0, m0 + NT_ // 2):
                st["proj", m, which, c] = True
                if which != 1:
                    t = y[128 * (m - m0):128 * (m - m0 + 1)]
                    dst = qt_s if which == 0 else vt_s
                    dst[m, 64 * c:64 * (c + 1), :] = _u32((t * QSCALE if which == 0 else t).T)

        def skew(c):
            st["skew", b, c] = True
            if b:
                kl = k_s[HM * b - 32:HM * (b + 1), ch(c)]
            else:
                kl = jnp.concatenate([jnp.zeros((32, 128), U32), k_s[0:HM, ch(c)]], axis=0)
            rolled = [kl] + [pltpu.roll(kl, 32 * r, 1) for r in range(1, 4)]
            for i in range(4):
                t = rolled[-i % 4][0:HM]
                for g in range(1, 4):
                    t = jnp.where(quad == g, rolled[(g - i) % 4][32 * (g // 2):32 * (g // 2) + HM], t)
                ks_s[4 * c + i, HM * b:HM * (b + 1), :] = t

        def plain(which, c):
            def run():
                y = _dot(st["xn"], wqkv_s[:, ch(4 * which + c)])
                for r in range(2):
                    emit(which, c, r, y[HM * r:HM * (r + 1)])
            return (run, TM)

        def pair(which, c):
            if not fast:
                ts = [plain(which, 2 * c), plain(which, 2 * c + 1)]
            else:
                def both(r, y1, y2):
                    emit(which, 2 * c, r, y1)
                    emit(which, 2 * c + 1, r, y2)
                n = 2 * which + c
                ts = group(_strassen_steps(lambda i: _dot(st["lx"][i], rhs(rq_s, i, n)), both), TM // 4)
            if which == 1:
                ts += [(lambda: skew(2 * c), 0), (lambda: skew(2 * c + 1), 0)]
            return ts
        return (t_ln, 0), [[pair(w, c) for w in range(3)] for c in range(2)]

    def ffn_tasks(b):
        fo, fg, fd = [k in CFG["st"] and b >= CFG[k + "0"] for k in "ogd"]

        def t_t():
            while pending and pending[0][0] // NT_ <= b:
                t_pv(*pending.pop(0))
            if fo:
                put_lhs("lo", ot_s[b % 2].T)
            else:
                st["o"] = ot_s[b % 2].T.astype(BF16)

        def emit_h(c, r, y):
            h_s[b % 2, HM * r:HM * (r + 1), ch(c)] = x_s[TM * b + HM * r:TM * b + HM * (r + 1), ch(c)].astype(F32) + y

        def t_o(c):
            if fo:
                return group(_strassen_steps(
                    lambda i: _dot(st["lo"][i], rhs(ro_s, i, c)),
                    lambda r, y1, y2: (emit_h(2 * c, r, y1), emit_h(2 * c + 1, r, y2))), TM // 4)

            def run(cc):
                y = _dot(st["o"], wo_s[:, ch(cc)])
                for r in range(2):
                    emit_h(cc, r, y[HM * r:HM * (r + 1)])
            return [(lambda: run(2 * c), 256), (lambda: run(2 * c + 1), 256)]

        def t_ln():
            hn = _ln(h_s[b % 2])
            if fg:
                put_lhs("lh", hn)
            else:
                st["hn"] = hn.astype(BF16)

        def act(c, r, g, u):
            hg = 0.5 * g
            a = (hg + hg * jnp.tanh(hg)) * u
            if not fd:
                st["a", r] = a
                if ("a", 0) in st and ("a", 1) in st:
                    st["ab", c] = jnp.concatenate([st.pop(("a", 0)), st.pop(("a", 1))], axis=0).astype(BF16)
                return
            st["a", c % 2, r] = a
            if all(("a", i, j) in st for i in range(2) for j in range(2)):
                quads = [st.pop(("a", i, j)) for j in range(2) for i in range(2)]
                for i, l in enumerate(_strassen_lhs(*quads)):
                    st["la", i, c // 2] = l.astype(BF16)

        def t_gu(c):
            if fg:
                return group(_strassen_steps(
                    lambda i: _dot(st["lh"][i], rhs(rg_s, i, c)), lambda r, g, u: act(c, r, g, u)), TM // 4)

            def t_g():
                st["g"] = _dot(st["hn"], wg_s[:, ch(c)])

            def t_u():
                u, g = _dot(st["hn"], wu_s[:, ch(c)]), st.pop("g")
                for r in range(2):
                    act(c, r, g[128 * r:128 * (r + 1)], u[128 * r:128 * (r + 1)])
            return [(t_g, 256), (t_u, 256)]

        def emit_y(c, r, y):
            out_s[TM * b + HM * r:TM * b + HM * (r + 1), ch(c)] = (
                h_s[b % 2, HM * r:HM * (r + 1), ch(c)] + y).astype(out_s.dtype)

        def t_d(c):
            if fd:
                def prod(i):
                    ys = [_dot(st["la", i, k], rhs(rd_s, i, c, slice(64 * k, 64 * (k + 1)))) for k in range(F // 256)]
                    return sum(ys[1:], ys[0])
                steps = _strassen_steps(prod,
                                        lambda r, y1, y2: (emit_y(2 * c, r, y1), emit_y(2 * c + 1, r, y2)))
                return [(f, w * 7 * TM // 8) for f, w in steps]

            def run(cc, k0, k1):
                ys = [_dot(st["ab", k], wd_s[ch(k), ch(cc)]) for k in range(k0 // 128, k1 // 128)]
                y = sum(ys[1:], ys[0])
                y = y if k0 == 0 else y + st.pop("y")
                if k1 == F:
                    for r in range(2):
                        emit_y(cc, r, y[128 * r:128 * (r + 1)])
                else:
                    st["y"] = y
            ks = list(range(0, F, 512)) + [F]
            return [((lambda cc=cc, k0=k0, k1=k1: run(cc, k0, k1)), (k1 - k0) // 2)
                    for cc in (2 * c, 2 * c + 1) for k0, k1 in zip(ks, ks[1:])]
        return (t_t, 0), t_o(0) + t_o(1), (t_ln, 0), [t_gu(c) for c in range(F // 128)], t_d(0) + ([start(ocopy(b, 0))] if b == NB - 1 else []) + t_d(1) + [start(ocopy(b, 1))]

    def t_qk(m, l, i):
        assert ("proj", m, 0, l) in st and ("skew", m // NT_, l) in st
        z = jnp.zeros((8, 128), U32)
        tiles = []
        for h in range(2):
            qt = qt_s[m, 64 * l + 16 * i + 8 * h:64 * l + 16 * i + 8 * (h + 1), :]
            tiles.append(jnp.concatenate([qt & quad_bits[g] if e == h else z for g in range(4) for e in range(2)], axis=0))
        qbd = _bf(jnp.concatenate(tiles, axis=1))
        t0 = 64 * m + 32
        if m < W // 128:
            kk = ks_s[4 * l + i, 0:t0 + 32, :]
        else:
            corner = jnp.where(quad % 2 == 1, ks_s[4 * l + i, t0 + 16:t0 + 32, :],
                               ks_s[4 * l + i, t0 - 128:t0 - 112, :])
            kk = jnp.concatenate([corner, ks_s[4 * l + i, t0 - 112:t0 + 16, :]], axis=0)
        st["s", m, l, i] = _dot(_bf(kk), qbd)

        if CFG["maxpos"]:
            t_max(m, l, 2 * i)
            t_max(m, l, 2 * i + 1)

    def t_max(m, l, hl):
        s = st["s", m, l, hl // 2][:, ch(hl % 2)]
        if m < W // 128:
            n = s.shape[0]
            mid = [s[64:n - 64]] if n > 128 else []
            s = jnp.concatenate([jnp.where(late, s[:64], -1e9)] + mid + [jnp.where(new_tri, s[n - 64:], -1e9)], axis=0)
        else:
            edge = jnp.where(new_tri, jnp.concatenate([s[W:], s[:32]], axis=0), s[:64])
            s = jnp.concatenate([edge, s[64:W]], axis=0)
        st["m", m, l, hl] = s, jnp.max(s, axis=0, keepdims=True)

    def t_sm(m, l, hl):
        if not CFG["maxpos"]:
            t_max(m, l, hl)
        s, mx = st.pop(("m", m, l, hl))
        e = p = jnp.exp2(s - mx)
        st["l", m, l, hl] = jnp.sum(e, axis=0, keepdims=True) if CFG["sumpos"] == 0 else e
        if m >= W // 128:
            p = jnp.concatenate([jnp.where(new_tri, 0.0, e[:64]), e[64:], jnp.where(new_tri, e[:64], 0.0)], axis=0)
        r = p.shape[0]
        parts = [jnp.where(late, p[:r - 64], p[64:]), jnp.where(late, p[r - 64:], 0.0)]
        if m >= W // 128:
            parts = [jnp.where(late, 0.0, p[:64])] + parts
        st["p", m, l, hl] = jnp.concatenate(parts, axis=0).astype(BF16)
        if CFG["sumpos"] == 1:
            st["l", m, l, hl] = jnp.sum(e, axis=0, keepdims=True)

    def t_pv(m, l, hl):
        pt = st.pop(("p", m, l, hl))
        assert ("proj", m, 2, l) in st
        nt = pt.shape[0] // 128
        r0 = 128 * l + DH * hl
        vt = _bf(jnp.concatenate([vt_s[m + 1 - nt + t, r0 // 2:(r0 + DH) // 2, :] for t in range(nt)], axis=1))
        o, tot = _dot(vt, pt), st.pop(("l", m, l, hl))
        if CFG["sumpos"] == 2:
            tot = jnp.sum(tot, axis=0, keepdims=True)
        o = o * (1.0 / tot)
        ot_s[m // NT_ % 2, r0:r0 + DH, ch(m % NT_)] = o

    heads = [(m, l, hl) for m in range(S // 128) for l in range(4) for hl in range(8)]
    heads[:64] = sorted(heads[:64], key=lambda t: (t[1] // 2, t[0]))
    HB = len(heads) // NB

    def merge(b, dense):
        total = sum(c for _, c in dense)
        done, spent = 0, 0
        qs, ahead = CFG["qs"], CFG["ahead"]
        for i in range(HB):
            n = HB * b + i
            if n % qs == 0:
                for k in range(0 if n == 0 else n + ahead, min(n + ahead + qs, len(heads)), 2):
                    t_qk(heads[k][0], heads[k][1], heads[k][2] // 2)
            if CFG["smpos"] == 0:
                t_sm(*heads[n])
            while done < len(dense) and spent + dense[done][1] / 2 <= total * (i + 1) / (HB - (ahead + qs if b == 0 else 0)):
                dense[done][0]()
                spent += dense[done][1]
                done += 1
            if CFG["smpos"] == 1:
                t_sm(*heads[n])
            pending.append(heads[n])
            while len(pending) > CFG["lag"] + (CFG["smpos"] == 2):
                t_pv(*pending.pop(0))
            if CFG["smpos"] == 2:
                t_sm(*heads[n])
        for fn, _ in dense[done:]:
            fn()

    def start(*cs):
        return (lambda: [c.start() for c in cs] and None, 0)

    def wait(*cs):
        def run():
            with _scope("wait"):
                for c in cs:
                    c.wait()
        return (run, 0)

    for c in (c_x0, c_qkv[0][1], c_qkv[0][0], c_qkv[0][2]):
        c.start()
    on = lambda k: k in CFG["st"]
    prep_q = [prep_cols(rq_s, n, wqkv_s, 2 * n, wqkv_s, 2 * n + 1) for n in range(6)] if on("q") else []
    prep_o = [prep_cols(ro_s, c, wo_s, 2 * c, wo_s, 2 * c + 1) for c in range(2)] if on("o") else []
    prep_g = [prep_cols(rg_s, c, wg_s, c, wu_s, c) for c in range(F // 128)] if on("g") else []
    prep_d = [prep_rhs(rd_s, slice(64 * k, 64 * (k + 1)), c, *[
        (lambda i=i, j=j, k=k, c=c: wd_s[ch(2 * k + i), ch(2 * c + j)]) for i in range(2) for j in range(2)])
        for c in range(2) for k in range(F // 256)] if on("d") else []

    def spread(ts, extra):
        out, done = [], 0
        for n, t in enumerate(ts):
            want = -(-(n + 1) * len(extra) // len(ts))
            out += extra[done:want] + [t]
            done = want
        return out

    def proj(b):
        if b >= NB:
            return []
        t_ln, ts = proj_tasks(b)
        return [t_ln] + [t for w in (1, 0, 2) for c in range(2) for t in ts[c][w]]

    t_ln, ts = proj_tasks(0)
    (q0, k0, v0), (q1, k1, v1) = c_qkv
    early = CFG["pq"]
    with_prep = lambda c, w: ts[c][w][:1] + ([prep_q[2 * w + c]] if early else []) + ts[c][w][1:]
    pro = [wait(c_x0), start(k1, q1, v1, c_x1), t_ln, wait(k0, q0, v0), start(c_wo, c_wg, c_wu)]
    pro += with_prep(0, 1) + with_prep(0, 0) + with_prep(0, 2)
    pro2 = [wait(k1, q1, v1, c_x1), start(c_wd, c_x2)] + with_prep(1, 1) + with_prep(1, 0) + with_prep(1, 2)
    if not CFG["pm"]:
        pro, pro2 = pro + pro2, []
    with _scope("pro"):
        for fn, _ in pro:
            fn()
    PA = CFG["pa"]
    carry = []
    for b in range(NB + 1):
        if b >= 1:
            pj = proj(b + PA)
            t_t, t_o, t_ln2, gu, down = ffn_tasks(b - 1)
            dense = [wait(c_wo)] + prep_o if b == 1 and not CFG["po"] else []
            mid = CFG['mid']
            dense += pj[:CFG["pre"]] + [t_t] + t_o + [t_ln2] + pj[CFG["pre"]:CFG["pre"] + mid] + carry
            rest = pj[CFG["pre"] + mid:]
            for c, ts in enumerate(gu):
                if b == 1:
                    if c == 0:
                        dense += [wait(c_wg, c_wu) if CFG["pd"] else wait(c_wg, c_wu, c_wd), prep_g[0]]
                    if c + 1 < len(gu):
                        ts = spread(ts, [prep_g[c + 1]]) if CFG["pg"] else ts + [prep_g[c + 1]]
                    if c >= CFG["pd"]:
                        n, k = len(gu) - CFG["pd"], c - CFG["pd"]
                        ts = spread(ts, prep_d[k * len(prep_d) // n:(k + 1) * len(prep_d) // n])
                        ts = ([wait(c_wd)] if k == 0 and CFG["pd"] else []) + ts
                if prep_g and b == CFG["g0"]:
                    ts = spread(ts, [prep_g[c]])
                if prep_d and b == CFG["d0"] and b >= 2:
                    ts = spread(ts, [prep_d[c]])
                dense += ts + rest[c * len(rest) // len(gu):(c + 1) * len(rest) // len(gu)]
            if b == 1:
                if CFG["pd"] >= len(gu):
                    dense += [wait(c_wd)] + (prep_d if CFG["d0"] == 0 else [])
                down = spread(down, prep_d) if CFG["d0"] == 1 else down
                down = spread(down, prep_o) if CFG["o0"] == 1 else down
                down = down + [wait(c_x2)]
            keep = CFG["tail"] if b + PA >= NB - 1 and b < NB else 0
            dense, carry = dense + down[:len(down) - keep], down[len(down) - keep:]
        else:
            dense = list(pro2)
            for n in range(1, PA + 1):
                if not early:
                    dense += prep_q
                dense += proj(n)
            if CFG["po"]:
                dense = dense[:-CFG["po"]] + [wait(c_wo)] + spread(dense[-CFG["po"]:], prep_o)
        with _scope("b%d" % b):
            if b < NB:
                merge(b, dense)
            else:
                for fn, _ in dense:
                    fn()
    for b in range(NB):
        ocopy(b, 1).wait()
    ocopy(NB - 1, 0).wait()


@jax.jit
def pallas_sequential_preLN__sliding_block__swiglu_ffn__prompt_kernel(A_x, A_wqkv, A_wo, B_x, B_w_gate, B_w_up, B_w_down):
    del B_x
    TM = CFG['tm']
    NB = S // TM
    any_spec = pl.BlockSpec(memory_space=pl.ANY)
    out = pl.pallas_call(
        _kernel,
        out_shape=jax.ShapeDtypeStruct((S, D), A_x.dtype),
        in_specs=[any_spec] * 6,
        out_specs=any_spec,
        scratch_shapes=[
            pltpu.VMEM((S, D), BF16), pltpu.VMEM((D, 3 * D), BF16), pltpu.VMEM((D, D), BF16),
            pltpu.VMEM((D, F), BF16), pltpu.VMEM((D, F), BF16), pltpu.VMEM((F, D), BF16),
            pltpu.VMEM((S, D), A_x.dtype),
            pltpu.VMEM((S // 128, D // 2, 128), U32), pltpu.VMEM((S // 2, D), U32),
            pltpu.VMEM((16, S // 2, 128), U32), pltpu.VMEM((S // 128, D // 2, 128), U32),
            pltpu.VMEM((2, D, TM), F32), pltpu.VMEM((2, TM, D), F32),
            pltpu.VMEM((7, D // 4, 3 * D // 2), U32), pltpu.VMEM((7, D // 4, D // 2), U32),
            pltpu.VMEM((7, D // 4, F), U32), pltpu.VMEM((7, F // 4, D // 2), U32),
            pltpu.SemaphoreType.DMA((13,)), pltpu.SemaphoreType.DMA((NB + 1,)),
        ],
        compiler_params=pltpu.CompilerParams(vmem_limit_bytes=64 * 1024 * 1024, flags=CFG.get("flags")),
    )(A_x.reshape(S, D), A_wqkv, A_wo, B_w_gate, B_w_up, B_w_down)
    return out.reshape(1, S, D)
```

```python
import numpy as np
import jax
import jax.numpy as jnp
from jax import lax
import jax.experimental.pallas as pl
import jax.experimental.pallas.tpu as pltpu

S, D, F, DH, W = 2048, 512, 1792, 16, 256
TM = 256
NB = S // TM
HB = 64
AHEAD = 8
EPS = 1e-5
QSCALE = float(DH ** -0.5 * np.log2(np.e))
F32, BF16, U32 = jnp.float32, jnp.bfloat16, jnp.uint32


def _ln(x):
    m = jnp.mean(x, axis=-1, keepdims=True)
    c = x - m
    v = jnp.mean(c * c, axis=-1, keepdims=True)
    return c * lax.rsqrt(v + EPS)


def _u32(x):
    return pltpu.bitcast(x.astype(BF16), U32)


def _bf(x):
    return pltpu.bitcast(x, BF16)


def _dot(a, b):
    return jnp.dot(a, b, preferred_element_type=F32)


def _ch(c):
    return slice(128 * c, 128 * (c + 1))


def _strassen_lhs(a11, a12, a21, a22):
    return [l.astype(BF16) for l in [a11 + a22, a21 + a22, a11, a22, a11 + a12, a21 - a11, a12 - a22]]


def _strassen_rhs(b11, b12, b21, b22):
    f11, f12, f21, f22 = [b.astype(F32) for b in (b11, b12, b21, b22)]
    return [r.astype(BF16) for r in [f11 + f22, b11, f12 - f22, f21 - f11, b22, f11 + f12, f21 + f22]]


def _strassen_steps(prod, emit):
    c = {}

    def s61():
        m6 = prod(5)
        c[1] = prod(0)
        c["t"] = c[1] + m6

    def s23():
        c[2], c[3] = prod(1), prod(2)
        c[22] = c.pop("t") - c[2] + c[3]

    def s47():
        m4 = prod(3)
        c["u"] = c.pop(1) + m4 + prod(6)
        emit(1, c.pop(2) + m4, c.pop(22))

    def s5():
        m5 = prod(4)
        emit(0, c.pop("u") - m5, c.pop(3) + m5)
    return [(s61, 2), (s23, 2), (s47, 2), (s5, 1)]


def _pairs(steps):
    def unit(ss):
        def run():
            for f, _ in ss:
                f()
        return run, 64 * sum(w for _, w in ss)
    return [unit(steps[k:k + 2]) for k in range(0, len(steps), 2)]


def _spread(tasks, extra):
    out, done = [], 0
    for n, t in enumerate(tasks):
        want = -(-(n + 1) * len(extra) // len(tasks))
        out += extra[done:want] + [t]
        done = want
    return out


def _start(*copies):
    def run():
        for c in copies:
            c.start()
    return run, 0


def _wait(*copies):
    def run():
        for c in copies:
            c.wait()
    return run, 0


def _kernel(x_hbm, wqkv_hbm, wo_hbm, wg_hbm, wu_hbm, wd_hbm, out_hbm,
            x_s, wqkv_s, wo_s, wg_s, wu_s, wd_s, out_s, qt_s, k_s, ks_s, vt_s, ot_s, h_s, sems):
    nsem = [0]

    def copy(src, dst):
        nsem[0] += 1
        return pltpu.make_async_copy(src, dst, sems.at[nsem[0] - 1])

    def rows(b, n=1):
        return pl.ds(b * TM, n * TM)

    c_x0, c_x1, c_x2 = [copy(x_hbm.at[r], x_s.at[r]) for r in (rows(0), rows(1, 2), rows(3, NB - 3))]
    (q0, k0, v0), (q1, k1, v1) = [
        [copy(wqkv_hbm.at[:, cs], wqkv_s.at[:, cs]) for cs in [pl.ds(D * w + 256 * c, 256) for w in range(3)]]
        for c in range(2)]
    c_wo, c_wd, c_wg, c_wu = copy(wo_hbm, wo_s), copy(wd_hbm, wd_s), copy(wg_hbm, wg_s), copy(wu_hbm, wu_s)
    c_out = [copy(out_s.at[rows(b)], out_hbm.at[rows(b)]) for b in range(NB - 1)]
    c_last = [copy(out_s.at[rows(NB - 1), cs], out_hbm.at[rows(NB - 1), cs])
              for cs in (pl.ds(0, 256), pl.ds(256, 256))]

    lane = lax.broadcasted_iota(jnp.int32, (1, 128), 1)
    quad = lane // 32
    quad_bits = [jnp.where(quad == g, np.uint32(0xFFFFFFFF), np.uint32(0)) for g in range(4)]
    odd = quad % 2 == 1
    late = lane >= 64
    row = lax.broadcasted_iota(jnp.int32, (64, 128), 0)
    col = lax.broadcasted_iota(jnp.int32, (64, 128), 1) % 64
    new_tri = row <= col
    st = {}

    def put_lhs(name, a):
        st[name] = _strassen_lhs(a[:128, :D // 2], a[:128, D // 2:], a[128:, :D // 2], a[128:, D // 2:])

    def prep(name, *quads):
        def run():
            st[name] = _strassen_rhs(*[ref[r, c] for ref, r, c in quads])
        return run, 0

    def prep_cols(name, w1, c1, w2, c2):
        lo, hi = slice(0, D // 2), slice(D // 2, D)
        return prep(name, (w1, lo, _ch(c1)), (w2, lo, _ch(c2)), (w1, hi, _ch(c1)), (w2, hi, _ch(c2)))

    def emit_qkv(b, which, c, r, y):
        m = 2 * b + r
        if which == 1:
            k_s[64 * m:64 * (m + 1), _ch(c)] = _u32(y)
        else:
            dst = qt_s if which == 0 else vt_s
            dst[m, 64 * c:64 * (c + 1), :] = _u32((y * QSCALE if which == 0 else y).T)

    def skew(b, c):
        def run():
            if b:
                kl = k_s[128 * b - 32:128 * (b + 1), _ch(c)]
            else:
                kl = jnp.concatenate([jnp.zeros((32, 128), U32), k_s[0:128, _ch(c)]], axis=0)
            both = (jnp.where(odd, pltpu.roll(kl, 32, 1), kl), jnp.where(odd, kl, pltpu.roll(kl, 96, 1)))
            for i, t in enumerate(both):
                swapped = pltpu.roll(t, 64, 1)
                ks_s[4 * c + i, _ch(b), :] = jnp.where(late, swapped[32:], t[:128])
                ks_s[4 * c + i + 2, _ch(b), :] = jnp.where(late, t[32:], swapped[:128])
        return run, 0

    def first_ln():
        xn = _ln(x_s[rows(0), :].astype(F32))
        st["xn"] = [xn[_ch(r)].astype(BF16) for r in range(2)]

    def first_proj(which, c):
        def plain(cc):
            def run():
                for r in range(2):
                    emit_qkv(0, which, cc, r, _dot(st["xn"][r], wqkv_s[:, _ch(4 * which + cc)]))
            return run, TM
        n = 2 * which + c
        ts = [plain(2 * c), prep_cols(("rq", n), wqkv_s, 2 * n, wqkv_s, 2 * n + 1), plain(2 * c + 1)]
        return ts + ([skew(0, 2 * c), skew(0, 2 * c + 1)] if which == 1 else [])

    def proj_tasks(b):
        def t_ln():
            put_lhs("lx", _ln(x_s[rows(b), :].astype(F32)))

        def steps(which, c):
            def emit(r, y1, y2):
                emit_qkv(b, which, 2 * c, r, y1)
                emit_qkv(b, which, 2 * c + 1, r, y2)
            return _strassen_steps(lambda i: _dot(st["lx"][i], st["rq", 2 * which + c][i]), emit)
        k, q, v = [_pairs(steps(w, 0) + steps(w, 1)) for w in (1, 0, 2)]
        return [(t_ln, 0)] + k + [skew(b, c) for c in range(4)] + q + v

    def ffn_tasks(b):
        def t_o():
            put_lhs("lo", ot_s[b % 2].T)

        def wo_steps(c):
            def emit(r, *ys):
                for cc, y in zip((2 * c, 2 * c + 1), ys):
                    h_s[b % 2, _ch(r), _ch(cc)] = x_s[_ch(2 * b + r), _ch(cc)].astype(F32) + y
            return _strassen_steps(lambda i: _dot(st["lo"][i], st["ro", c][i]), emit)

        def t_ln():
            put_lhs("lh", _ln(h_s[b % 2]))

        def gu_steps(c):
            def emit(r, g, u):
                hg = 0.5 * g
                st["a", c % 2, r] = (hg + hg * jnp.tanh(hg)) * u
                if c % 2 == 1 and r == 0:
                    st["la", c // 2] = _strassen_lhs(*[st.pop(("a", i, j)) for j in range(2) for i in range(2)])
            return _strassen_steps(lambda i: _dot(st["lh"][i], st["rg", c][i]), emit)

        def down_tasks(c):
            def prod(i):
                ys = [_dot(st["la", k][i], st["rd", c, k][i]) for k in range(F // 256)]
                return sum(ys[1:], ys[0])

            def emit(r, *ys):
                for cc, y in zip((2 * c, 2 * c + 1), ys):
                    out_s[_ch(2 * b + r), _ch(cc)] = (h_s[b % 2, _ch(r), _ch(cc)] + y).astype(out_s.dtype)
            return [(f, 224 * w) for f, w in _strassen_steps(prod, emit)]
        if b < NB - 1:
            down = down_tasks(0) + down_tasks(1) + [_start(c_out[b])]
        else:
            down = down_tasks(0) + [_start(c_last[0])] + down_tasks(1) + [_start(c_last[1])]
        return ([(t_o, 0)] + _pairs(wo_steps(0) + wo_steps(1)) + [(t_ln, 0)],
                [_pairs(gu_steps(2 * c) + gu_steps(2 * c + 1)) for c in range(F // 256)], down)

    def scores(m, l, i):
        z = jnp.zeros((8, 128), U32)
        tiles = []
        for h in range(2):
            qt = qt_s[m, 64 * l + 16 * i + 8 * h:64 * l + 16 * i + 8 * (h + 1), :]
            tiles.append(jnp.concatenate(
                [qt & quad_bits[g] if e == h else z for g in range(4) for e in range(2)], axis=0))
        qbd = _bf(jnp.concatenate(tiles, axis=1))
        t0 = 64 * m + 32
        if m < W // 128:
            kk = ks_s[4 * l + i, 0:t0 + 32, :]
        else:
            corner = jnp.where(odd, ks_s[4 * l + i, t0 + 16:t0 + 32, :], ks_s[4 * l + i, t0 - 128:t0 - 112, :])
            kk = jnp.concatenate([corner, ks_s[4 * l + i, t0 - 112:t0 + 16, :]], axis=0)
        both = _dot(_bf(kk), qbd)
        for h in range(2):
            s = both[:, _ch(h)]
            if m < W // 128:
                n = s.shape[0]
                mid = [s[64:n - 64]] if n > 128 else []
                s = jnp.concatenate(
                    [jnp.where(late, s[:64], -1e9)] + mid + [jnp.where(new_tri, s[n - 64:], -1e9)], axis=0)
            else:
                edge = jnp.where(new_tri, jnp.concatenate([s[W:], s[:32]], axis=0), s[:64])
                s = jnp.concatenate([edge, s[64:W]], axis=0)
            st["s", m, l, 2 * i + h] = s, jnp.max(s, axis=0, keepdims=True)

    def attend(m, l, hl):
        s, mx = st.pop(("s", m, l, hl))
        p = e = jnp.exp2(s - mx)
        tot = jnp.sum(e, axis=0, keepdims=True)
        if m >= W // 128:
            old = jnp.where(new_tri, 0.0, e[:64])
            p = jnp.concatenate([old, e[64:], jnp.where(new_tri, e[:64], 0.0)], axis=0)
        r = p.shape[0]
        parts = [jnp.where(late, p[:r - 64], p[64:]), jnp.where(late, p[r - 64:], 0.0)]
        if m >= W // 128:
            parts = [jnp.where(late, 0.0, p[:64])] + parts
        pt = jnp.concatenate(parts, axis=0).astype(BF16)
        nt = pt.shape[0] // 128
        r0 = 128 * l + DH * hl
        vt = _bf(jnp.concatenate([vt_s[m + 1 - nt + t, r0 // 2:(r0 + DH) // 2, :] for t in range(nt)], axis=1))
        ot_s[m // 2 % 2, r0:r0 + DH, _ch(m % 2)] = _dot(vt, pt) * (1.0 / tot)

    heads = [(m, l, hl) for m in range(S // 128) for l in range(4) for hl in range(8)]
    heads[:HB] = sorted(heads[:HB], key=lambda t: (t[1] // 2, t[0]))

    def merge(b, dense):
        total = sum(c for _, c in dense)
        span = HB - (AHEAD + 4 if b == 0 else 0)
        done, spent = 0, 0
        for i in range(HB):
            n = HB * b + i
            if n % 4 == 0:
                for k in range(n + AHEAD if n else 0, min(n + AHEAD + 4, len(heads)), 2):
                    scores(heads[k][0], heads[k][1], heads[k][2] // 2)
            while done < len(dense) and spent + dense[done][1] / 2 <= total * (i + 1) / span:
                dense[done][0]()
                spent += dense[done][1]
                done += 1
            attend(*heads[n])
        for fn, _ in dense[done:]:
            fn()

    prep_o = [prep_cols(("ro", c), wo_s, 2 * c, wo_s, 2 * c + 1) for c in range(2)]
    prep_g = [prep_cols(("rg", c), wg_s, c, wu_s, c) for c in range(F // 128)]
    prep_d = [prep(("rd", c, k), *[(wd_s, _ch(2 * k + i), _ch(2 * c + j)) for i in range(2) for j in range(2)])
              for c in range(2) for k in range(F // 256)]

    for fn, _ in ([_start(c_x0, k0, q0, v0), _wait(c_x0), _start(k1, q1, v1, c_x1), (first_ln, 0),
                   _wait(k0, q0, v0), _start(c_wo, c_wg, c_wu)]
                  + first_proj(1, 0) + first_proj(0, 0) + first_proj(2, 0)):
        fn()
    merge(0, [_wait(k1, q1, v1, c_x1), _start(c_wd, c_x2)]
          + first_proj(1, 1) + first_proj(0, 1) + first_proj(2, 1) + proj_tasks(1))
    carry = []
    for b in range(1, NB + 1):
        pj = proj_tasks(b + 1) if b + 1 < NB else []
        wo, gu, down = ffn_tasks(b - 1)
        dense = [_wait(c_wo)] + prep_o if b == 1 else []
        dense += pj[:3] + wo + pj[3:7] + carry
        rest = pj[7:]
        for c, ts in enumerate(gu):
            if b == 1:
                if c == 0:
                    dense += [_wait(c_wg, c_wu, c_wd)] + prep_g[:2]
                ts = _spread(ts, prep_g[2 * c + 2:2 * c + 4] + prep_d[2 * c:2 * c + 2])
            dense += ts + rest[c * len(rest) // len(gu):(c + 1) * len(rest) // len(gu)]
        if b == 1:
            down = down + [_wait(c_x2)]
        keep = 3 if NB - 2 <= b < NB else 0
        dense, carry = dense + down[:len(down) - keep], down[len(down) - keep:]
        if b < NB:
            merge(b, dense)
        else:
            for fn, _ in dense:
                fn()
    for c in c_out + c_last:
        c.wait()


@jax.jit
def pallas_sequential_preLN__sliding_block__swiglu_ffn__prompt_kernel(
    A_x: jax.Array,
    A_wqkv: jax.Array,
    A_wo: jax.Array,
    B_x: jax.Array,
    B_w_gate: jax.Array,
    B_w_up: jax.Array,
    B_w_down: jax.Array,
):
    del B_x
    hbm = pl.BlockSpec(memory_space=pl.ANY)
    out = pl.pallas_call(
        _kernel,
        out_shape=jax.ShapeDtypeStruct((S, D), A_x.dtype),
        in_specs=[hbm] * 6,
        out_specs=hbm,
        scratch_shapes=[
            pltpu.VMEM((S, D), BF16), pltpu.VMEM((D, 3 * D), BF16), pltpu.VMEM((D, D), BF16),
            pltpu.VMEM((D, F), BF16), pltpu.VMEM((D, F), BF16), pltpu.VMEM((F, D), BF16),
            pltpu.VMEM((S, D), A_x.dtype),
            pltpu.VMEM((S // 128, D // 2, 128), U32), pltpu.VMEM((S // 2, D), U32),
            pltpu.VMEM((16, S // 2, 128), U32), pltpu.VMEM((S // 128, D // 2, 128), U32),
            pltpu.VMEM((2, D, TM), F32), pltpu.VMEM((2, TM, D), F32),
            pltpu.SemaphoreType.DMA((13 + NB + 1,)),
        ],
        compiler_params=pltpu.CompilerParams(
            vmem_limit_bytes=64 * 1024 * 1024, flags={"XLA_TPU_FORCE_LP_LLO_SCHEDULER": True}),
    )(A_x.reshape(S, D), A_wqkv, A_wo, B_w_gate, B_w_up, B_w_down)
    return out.reshape(1, S, D)
```

```python
import numpy as np
import jax
import jax.numpy as jnp
from jax import lax
import jax.experimental.pallas as pl
import jax.experimental.pallas.tpu as pltpu

S, D, F, DH, W = 2048, 512, 1792, 16, 256
TM = 256
NB = S // TM
HB = 64
AHEAD = 8
EPS = 1e-5
QSCALE = float(DH ** -0.5 * np.log2(np.e))
F32, BF16, U32 = jnp.float32, jnp.bfloat16, jnp.uint32


def _ln(x):
    m = jnp.mean(x, axis=-1, keepdims=True)
    c = x - m
    v = jnp.mean(c * c, axis=-1, keepdims=True)
    return c * lax.rsqrt(v + EPS)


def _u32(x):
    return pltpu.bitcast(x.astype(BF16), U32)


def _bf(x):
    return pltpu.bitcast(x, BF16)


def _dot(a, b):
    return jnp.dot(a, b, preferred_element_type=F32)


def _ch(c):
    return slice(128 * c, 128 * (c + 1))


def _strassen_lhs(a11, a12, a21, a22):
    return [l.astype(BF16) for l in [a11 + a22, a21 + a22, a11, a22, a11 + a12, a21 - a11, a12 - a22]]


def _strassen_rhs(b11, b12, b21, b22):
    f11, f12, f21, f22 = [b.astype(F32) for b in (b11, b12, b21, b22)]
    return [r.astype(BF16) for r in [f11 + f22, b11, f12 - f22, f21 - f11, b22, f11 + f12, f21 + f22]]


def _strassen_steps(prod, emit):
    c = {}

    def s61():
        m6 = prod(5)
        c[1] = prod(0)
        c["t"] = c[1] + m6

    def s23():
        c[2], c[3] = prod(1), prod(2)
        c[22] = c.pop("t") - c[2] + c[3]

    def s47():
        m4 = prod(3)
        c["u"] = c.pop(1) + m4 + prod(6)
        emit(1, c.pop(2) + m4, c.pop(22))

    def s5():
        m5 = prod(4)
        emit(0, c.pop("u") - m5, c.pop(3) + m5)
    return [(s61, 2), (s23, 2), (s47, 2), (s5, 1)]


def _pairs(steps):
    def unit(ss):
        def run():
            for f, _ in ss:
                f()
        return run, 64 * sum(w for _, w in ss)
    return [unit(steps[k:k + 2]) for k in range(0, len(steps), 2)]


def _spread(tasks, extra):
    out, done = [], 0
    for n, t in enumerate(tasks):
        want = -(-(n + 1) * len(extra) // len(tasks))
        out += extra[done:want] + [t]
        done = want
    return out


def _start(*copies):
    def run():
        for c in copies:
            c.start()
    return run, 0


def _wait(*copies):
    def run():
        for c in copies:
            c.wait()
    return run, 0


def _kernel(x_hbm, wqkv_hbm, wo_hbm, wg_hbm, wu_hbm, wd_hbm, out_hbm,
            x_s, wqkv_s, wo_s, wg_s, wu_s, wd_s, out_s, qt_s, k_s, ks_s, vt_s, ot_s, h_s, sems):
    nsem = [0]

    def copy(src, dst):
        nsem[0] += 1
        return pltpu.make_async_copy(src, dst, sems.at[nsem[0] - 1])

    def rows(b, n=1):
        return pl.ds(b * TM, n * TM)

    c_x0, c_x1, c_x2 = [copy(x_hbm.at[r], x_s.at[r]) for r in (rows(0), rows(1, 2), rows(3, NB - 3))]
    (q0, k0, v0), (q1, k1, v1) = [
        [copy(wqkv_hbm.at[:, cs], wqkv_s.at[:, cs]) for cs in [pl.ds(D * w + 256 * c, 256) for w in range(3)]]
        for c in range(2)]
    c_wo, c_wd, c_wg, c_wu = copy(wo_hbm, wo_s), copy(wd_hbm, wd_s), copy(wg_hbm, wg_s), copy(wu_hbm, wu_s)
    c_out = [copy(out_s.at[rows(b)], out_hbm.at[rows(b)]) for b in range(NB - 1)]
    c_last = [copy(out_s.at[rows(NB - 1), cs], out_hbm.at[rows(NB - 1), cs])
              for cs in (pl.ds(0, 256), pl.ds(256, 256))]

    lane = lax.broadcasted_iota(jnp.int32, (1, 128), 1)
    quad = lane // 32
    quad_bits = [jnp.where(quad == g, np.uint32(0xFFFFFFFF), np.uint32(0)) for g in range(4)]
    odd = quad % 2 == 1
    late = lane >= 64
    row = lax.broadcasted_iota(jnp.int32, (64, 128), 0)
    col = lax.broadcasted_iota(jnp.int32, (64, 128), 1) % 64
    new_tri = row <= col
    st = {}

    def put_lhs(name, a):
        st[name] = _strassen_lhs(a[:128, :D // 2], a[:128, D // 2:], a[128:, :D // 2], a[128:, D // 2:])

    def prep(name, *quads):
        def run():
            st[name] = _strassen_rhs(*[ref[r, c] for ref, r, c in quads])
        return run, 0

    def prep_cols(name, w1, c1, w2, c2):
        lo, hi = slice(0, D // 2), slice(D // 2, D)
        return prep(name, (w1, lo, _ch(c1)), (w2, lo, _ch(c2)), (w1, hi, _ch(c1)), (w2, hi, _ch(c2)))

    def emit_qkv(b, which, c, r, y):
        m = 2 * b + r
        if which == 1:
            k_s[64 * m:64 * (m + 1), _ch(c)] = _u32(y)
        else:
            dst = qt_s if which == 0 else vt_s
            dst[m, 64 * c:64 * (c + 1), :] = _u32((y * QSCALE if which == 0 else y).T)

    def skew(b, c):
        def run():
            if b:
                kl = k_s[128 * b - 32:128 * (b + 1), _ch(c)]
            else:
                kl = jnp.concatenate([jnp.zeros((32, 128), U32), k_s[0:128, _ch(c)]], axis=0)
            both = (jnp.where(odd, pltpu.roll(kl, 32, 1), kl), jnp.where(odd, kl, pltpu.roll(kl, 96, 1)))
            for i, t in enumerate(both):
                swapped = pltpu.roll(t, 64, 1)
                ks_s[4 * c + i, _ch(b), :] = jnp.where(late, swapped[32:], t[:128])
                ks_s[4 * c + i + 2, _ch(b), :] = jnp.where(late, t[32:], swapped[:128])
        return run, 0

    def first_ln():
        xn = _ln(x_s[rows(0), :].astype(F32))
        st["xn"] = [xn[_ch(r)].astype(BF16) for r in range(2)]

    def first_proj(which, c):
        def plain(cc):
            def run():
                for r in range(2):
                    emit_qkv(0, which, cc, r, _dot(st["xn"][r], wqkv_s[:, _ch(4 * which + cc)]))
            return run, TM
        n = 2 * which + c
        ts = [plain(2 * c), prep_cols(("rq", n), wqkv_s, 2 * n, wqkv_s, 2 * n + 1), plain(2 * c + 1)]
        return ts + ([skew(0, 2 * c), skew(0, 2 * c + 1)] if which == 1 else [])

    def proj_tasks(b):
        def t_ln():
            put_lhs("lx", _ln(x_s[rows(b), :].astype(F32)))

        def steps(which, c):
            def emit(r, y1, y2):
                emit_qkv(b, which, 2 * c, r, y1)
                emit_qkv(b, which, 2 * c + 1, r, y2)
            return _strassen_steps(lambda i: _dot(st["lx"][i], st["rq", 2 * which + c][i]), emit)
        k, q, v = [_pairs(steps(w, 0) + steps(w, 1)) for w in (1, 0, 2)]
        return [(t_ln, 0)] + k + [skew(b, c) for c in range(4)] + q + v

    def ffn_tasks(b):
        def t_o():
            put_lhs("lo", ot_s[b % 2].T)

        def wo_steps(c):
            def emit(r, *ys):
                for cc, y in zip((2 * c, 2 * c + 1), ys):
                    h_s[b % 2, _ch(r), _ch(cc)] = x_s[_ch(2 * b + r), _ch(cc)].astype(F32) + y
            return _strassen_steps(lambda i: _dot(st["lo"][i], st["ro", c][i]), emit)

        def t_ln():
            put_lhs("lh", _ln(h_s[b % 2]))

        def gu_steps(c):
            def emit(r, g, u):
                hg = 0.5 * g
                st["a", c % 2, r] = (1.0 + jnp.tanh(hg)) * (hg * u)
                if c % 2 == 1 and r == 0:
                    st["la", c // 2] = _strassen_lhs(*[st.pop(("a", i, j)) for j in range(2) for i in range(2)])
            return _strassen_steps(lambda i: _dot(st["lh"][i], st["rg", c][i]), emit)

        def down_tasks(c):
            def prod(i):
                ys = [_dot(st["la", k][i], st["rd", c, k][i]) for k in range(F // 256)]
                return ((ys[0] + ys[1]) + (ys[2] + ys[3])) + ((ys[4] + ys[5]) + ys[6])

            def emit(r, *ys):
                for cc, y in zip((2 * c, 2 * c + 1), ys):
                    out_s[_ch(2 * b + r), _ch(cc)] = (h_s[b % 2, _ch(r), _ch(cc)] + y).astype(out_s.dtype)
            return [(f, 224 * w) for f, w in _strassen_steps(prod, emit)]
        if b < NB - 1:
            down = down_tasks(0) + down_tasks(1) + [_start(c_out[b])]
        else:
            down = down_tasks(0) + [_start(c_last[0])] + down_tasks(1) + [_start(c_last[1])]
        return ([(t_o, 0)] + _pairs(wo_steps(0) + wo_steps(1)) + [(t_ln, 0)],
                [_pairs(gu_steps(2 * c) + gu_steps(2 * c + 1)) for c in range(F // 256)], down)

    def scores(m, l, i):
        z = jnp.zeros((8, 128), U32)
        tiles = []
        for h in range(2):
            qt = qt_s[m, 64 * l + 16 * i + 8 * h:64 * l + 16 * i + 8 * (h + 1), :]
            tiles.append(jnp.concatenate(
                [qt & quad_bits[g] if e == h else z for g in range(4) for e in range(2)], axis=0))
        qbd = _bf(jnp.concatenate(tiles, axis=1))
        t0 = 64 * m + 32
        if m < W // 128:
            kk = ks_s[4 * l + i, 0:t0 + 32, :]
        else:
            corner = jnp.where(odd, ks_s[4 * l + i, t0 + 16:t0 + 32, :], ks_s[4 * l + i, t0 - 128:t0 - 112, :])
            kk = jnp.concatenate([corner, ks_s[4 * l + i, t0 - 112:t0 + 16, :]], axis=0)
        both = _dot(_bf(kk), qbd)
        for h in range(2):
            s = both[:, _ch(h)]
            if m < W // 128:
                n = s.shape[0]
                mid = [s[64:n - 64]] if n > 128 else []
                s = jnp.concatenate(
                    [jnp.where(late, s[:64], -1e9)] + mid + [jnp.where(new_tri, s[n - 64:], -1e9)], axis=0)
            else:
                edge = jnp.where(new_tri, jnp.concatenate([s[W:], s[:32]], axis=0), s[:64])
                s = jnp.concatenate([edge, s[64:W]], axis=0)
            st["s", m, l, 2 * i + h] = s, jnp.max(s, axis=0, keepdims=True)

    def attend(m, l, hl):
        s, mx = st.pop(("s", m, l, hl))
        p = e = jnp.exp2(s - mx)
        tot = jnp.sum(e, axis=0, keepdims=True)
        if m >= W // 128:
            old = jnp.where(new_tri, 0.0, e[:64])
            p = jnp.concatenate([old, e[64:], jnp.where(new_tri, e[:64], 0.0)], axis=0)
        r = p.shape[0]
        parts = [jnp.where(late, p[:r - 64], p[64:]), jnp.where(late, p[r - 64:], 0.0)]
        if m >= W // 128:
            parts = [jnp.where(late, 0.0, p[:64])] + parts
        pt = jnp.concatenate(parts, axis=0).astype(BF16)
        nt = pt.shape[0] // 128
        r0 = 128 * l + DH * hl
        vt = _bf(jnp.concatenate([vt_s[m + 1 - nt + t, r0 // 2:(r0 + DH) // 2, :] for t in range(nt)], axis=1))
        ot_s[m // 2 % 2, r0:r0 + DH, _ch(m % 2)] = _dot(vt, pt) * (1.0 / tot)

    heads = [(m, l, hl) for m in range(S // 128) for l in range(4) for hl in range(8)]
    heads[:HB] = sorted(heads[:HB], key=lambda t: (t[1] // 2, t[0]))

    def merge(b, dense):
        total = sum(c for _, c in dense)
        span = HB - (AHEAD + 4 if b == 0 else 0)
        done, spent = 0, 0
        for i in range(HB):
            n = HB * b + i
            if n % 4 == 0:
                for k in range(n + AHEAD if n else 0, min(n + AHEAD + 4, len(heads)), 2):
                    scores(heads[k][0], heads[k][1], heads[k][2] // 2)
            while done < len(dense) and spent + dense[done][1] / 2 <= total * (i + 1) / span:
                dense[done][0]()
                spent += dense[done][1]
                done += 1
            attend(*heads[n])
        for fn, _ in dense[done:]:
            fn()

    prep_o = [prep_cols(("ro", c), wo_s, 2 * c, wo_s, 2 * c + 1) for c in range(2)]
    prep_g = [prep_cols(("rg", c), wg_s, c, wu_s, c) for c in range(F // 128)]
    prep_d = [prep(("rd", c, k), *[(wd_s, _ch(2 * k + i), _ch(2 * c + j)) for i in range(2) for j in range(2)])
              for c in range(2) for k in range(F // 256)]

    for fn, _ in ([_start(c_x0, k0, q0, v0), _wait(c_x0), _start(k1, q1, v1, c_x1), (first_ln, 0),
                   _wait(k0, q0, v0), _start(c_wo, c_wg, c_wu)]
                  + first_proj(1, 0) + first_proj(0, 0) + first_proj(2, 0)):
        fn()
    merge(0, [_wait(k1, q1, v1, c_x1), _start(c_wd, c_x2)]
          + first_proj(1, 1) + first_proj(0, 1) + first_proj(2, 1) + proj_tasks(1))
    carry = []
    for b in range(1, NB + 1):
        pj = proj_tasks(b + 1) if b + 1 < NB else []
        wo, gu, down = ffn_tasks(b - 1)
        dense = [_wait(c_wo)] + prep_o if b == 1 else []
        dense += pj[:3] + wo + pj[3:7] + carry
        rest = pj[7:]
        for c, ts in enumerate(gu):
            if b == 1:
                if c == 0:
                    dense += [_wait(c_wg, c_wu, c_wd)] + prep_g[:2]
                ts = _spread(ts, prep_g[2 * c + 2:2 * c + 4] + prep_d[c:c + 1])
            dense += ts + rest[c * len(rest) // len(gu):(c + 1) * len(rest) // len(gu)]
        if b == 1:
            down = _spread(down[:4], prep_d[7:]) + down[4:] + [_wait(c_x2)]
        keep = 3 if NB - 2 <= b < NB else 0
        dense, carry = dense + down[:len(down) - keep], down[len(down) - keep:]
        if b < NB:
            merge(b, dense)
        else:
            for fn, _ in dense:
                fn()
    for c in c_out + c_last:
        c.wait()


@jax.jit
def pallas_sequential_preLN__sliding_block__swiglu_ffn__prompt_kernel(
    A_x: jax.Array,
    A_wqkv: jax.Array,
    A_wo: jax.Array,
    B_x: jax.Array,
    B_w_gate: jax.Array,
    B_w_up: jax.Array,
    B_w_down: jax.Array,
):
    del B_x
    hbm = pl.BlockSpec(memory_space=pl.ANY)
    out = pl.pallas_call(
        _kernel,
        out_shape=jax.ShapeDtypeStruct((S, D), A_x.dtype),
        in_specs=[hbm] * 6,
        out_specs=hbm,
        scratch_shapes=[
            pltpu.VMEM((S, D), BF16), pltpu.VMEM((D, 3 * D), BF16), pltpu.VMEM((D, D), BF16),
            pltpu.VMEM((D, F), BF16), pltpu.VMEM((D, F), BF16), pltpu.VMEM((F, D), BF16),
            pltpu.VMEM((S, D), A_x.dtype),
            pltpu.VMEM((S // 128, D // 2, 128), U32), pltpu.VMEM((S // 2, D), U32),
            pltpu.VMEM((16, S // 2, 128), U32), pltpu.VMEM((S // 128, D // 2, 128), U32),
            pltpu.VMEM((2, D, TM), F32), pltpu.VMEM((2, TM, D), F32),
            pltpu.SemaphoreType.DMA((13 + NB + 1,)),
        ],
        compiler_params=pltpu.CompilerParams(
            vmem_limit_bytes=64 * 1024 * 1024, flags={"XLA_TPU_FORCE_LP_LLO_SCHEDULER": True}),
    )(A_x.reshape(S, D), A_wqkv, A_wo, B_w_gate, B_w_up, B_w_down)
    return out.reshape(1, S, D)
```
